```python
import os as _os
_os.environ.setdefault("JAX_PLATFORMS", "cpu")
import jax
import jax.numpy as jnp

def _softmax(x, axis=-1):
    return jax.nn.softmax(x, axis=axis)
def _gelu(x):
    return jax.nn.gelu(x, approximate=True)
def _silu(x):
    return jax.nn.silu(x)
def _sigmoid(x):
    return jax.nn.sigmoid(x)
def _layernorm(x, axis=-1, eps=1e-5):
    m = jnp.mean(x, axis=axis, keepdims=True)
    v = jnp.var(x, axis=axis, keepdims=True)
    return (x - m) / jnp.sqrt(v + eps)
def _scatter_add(tgt, idx, src, axis=0):
    return tgt.at[idx].add(src)
def _segment_sum(src, seg, n):
    return jax.ops.segment_sum(src, seg, n)
class _Rng:
    def __init__(self, key):
        self._k = key
    def _next(self):
        self._k, sub = jax.random.split(self._k)
        return sub
    def normal(self, shape):
        return jax.random.normal(self._next(), shape, dtype=jnp.bfloat16)
    def randint(self, lo, hi, shape):
        return jax.random.randint(self._next(), shape, lo, hi, dtype=jnp.int32)
    def uniform(self, shape, lo=0.0, hi=1.0):
        return jax.random.uniform(self._next(), shape, jnp.bfloat16, lo, hi)
    def permutation(self, n):
        return jax.random.permutation(self._next(), n)


kernel_name = 'gated_mix__linear_attn_block__glu_gated_swiglu__prompt'

def setup_inputs():
    _rng = _Rng(jax.random.key(int.from_bytes(__import__("os").urandom(4), "little")))
    _w = (lambda a: (lambda t: t.astype(jnp.bfloat16) if jnp.issubdtype(t.dtype, jnp.floating) else t)(jnp.asarray(a)))
    def _A_setup():
        B, S, D = 1, 2048, 1024
        return {
            "x": _w((lambda *s: _rng.normal(s) * 0.05)(B, S, D)),
            "wqkv": _w((lambda *s: _rng.normal(s) * 0.8)(D, 3 * D)),
            "wo": _w((lambda *s: _rng.normal(s) * 0.05)(D, D)),
        }
    _A_in = _A_setup()

    def _B_setup():
        B, S, D, F = 1, 2048, 1024, 3584
        return {
            "x": _w((lambda *s: _rng.normal(s) * 0.05)(B, S, D)),
            "w1": _w((lambda *s: _rng.normal(s) * 1.6)(D, F) * (2.0 / D) ** 0.5),
            "w3": _w((lambda *s: _rng.normal(s) * 1.6)(D, F) * (2.0 / D) ** 0.5),
            "w2": _w((lambda *s: _rng.normal(s) * 1.6)(F, D) * (2.0 / F) ** 0.5),
        }
    _B_in = _B_setup()

    return {
        "A_x": _A_in["x"],
        "A_wqkv": _A_in["wqkv"],
        "A_wo": _A_in["wo"],
        "B_x": _B_in["x"],
        "B_w1": _B_in["w1"],
        "B_w3": _B_in["w3"],
        "B_w2": _B_in["w2"],
        "gate_w": _w((lambda *s: _rng.normal(s) * 0.05)(1024) * 16.0),
    }

def reference(A_x, A_wqkv, A_wo, B_x, B_w1, B_w3, B_w2, gate_w):
    def _A_ref(x, wqkv, wo):
        B, S, D = x.shape
        H = 32; Dh = D // H
        qkv = (lambda x, *d: x.transpose(*d))((x @ wqkv).reshape(B, S, 3, H, Dh), 2, 0, 3, 1, 4)
        q, k, v = qkv[0], qkv[1], qkv[2]
        phi = lambda t: jnp.where(t > 0, t + 1, jnp.exp(t)) + 1e-6
        pq, pk = phi(q), phi(k)
        kv = jnp.einsum("bhsd,bhse->bhde", pk, v)
        z = jnp.einsum("bhsd->bhd", pk)
        num = jnp.einsum("bhqd,bhde->bhqe", pq, kv)
        den = jnp.einsum("bhqd,bhd->bhq", pq, z)[..., None] + 1e-6
        o = num / den
        return (lambda x, *d: x.transpose(*d))(o, 0, 2, 1, 3).reshape(B, S, D) @ wo

    def _B_ref(x, w1, w3, w2):
        gate = jnp.einsum("bsd,df->bsf", x, w1)
        up = jnp.einsum("bsd,df->bsf", x, w3)
        h = _silu(gate) * up
        out = jnp.einsum("bsf,fd->bsd", h, w2)
        return out

    x = A_x
    g = _sigmoid((x * gate_w).sum(-1, keepdims=True))
    a = _A_ref(x, A_wqkv, A_wo)
    b = _B_ref(x, B_w1, B_w3, B_w2)
    return g * a + (1 - g) * b
```

```python
import functools
import contextlib
import jax
import jax.numpy as jnp
import jax.experimental.pallas as pl
import jax.experimental.pallas.tpu as pltpu

S, D, F, H = 2048, 1024, 3584, 32
DH = D // H
bf16, f32 = jnp.bfloat16, jnp.float32
NG = D // 128
NF = F // 128

def phi(t):
    return jnp.where(t > 0, t + 1.0, jnp.exp(t)) + 1e-6

def rcp(y):
    return pltpu.reciprocal(y, approx=True)

def sigmoid(x):
    return rcp(1.0 + jnp.exp(-x))

def dot(a, b):
    return jnp.dot(a, b, preferred_element_type=f32)

def cat(xs):
    return xs[0] if len(xs) == 1 else jnp.concatenate(xs, axis=1)

def make(TS1=512, TS2=128, FC=512, scopes=False, GW=1):
    n1 = S // TS1
    n2 = S // TS2
    nf = F // FC
    sc = (lambda n: jax.named_scope(n)) if scopes else (lambda n: contextlib.nullcontext())
    def kern(x_hbm, wqkv_hbm, wo_hbm, w1_hbm, w3_hbm, w2_hbm, gw_ref, o_hbm,
             x_v, wqkv_v, wo_v, w1_v, w3_v, w2_v, m_v, z_v, kv_v, zacc_v, o_v, sems, osems):
        def cp(src, dst, r0, nr, c0, nc, sem):
            return pltpu.make_async_copy(src.at[pl.ds(r0, nr), pl.ds(c0, nc)], dst.at[pl.ds(r0, nr), pl.ds(c0, nc)], sems.at[sem])
        xcp = [cp(x_hbm, x_v, i * TS1, TS1, 0, D, i) for i in range(n1)]
        b = n1
        NW = NG // GW
        kcp = [cp(wqkv_hbm, wqkv_v, 0, D, D + g * 128 * GW, 128 * GW, b + g) for g in range(NW)]
        b += NW
        vcp = [cp(wqkv_hbm, wqkv_v, 0, D, 2 * D + g * 128 * GW, 128 * GW, b + g) for g in range(NW)]
        b += NW
        c_wo = cp(wo_hbm, wo_v, 0, D, 0, D, b)
        c_q = cp(wqkv_hbm, wqkv_v, 0, D, 0, D, b + 1)
        c_w1 = cp(w1_hbm, w1_v, 0, D, 0, F, b + 2)
        c_w3 = cp(w3_hbm, w3_v, 0, D, 0, F, b + 3)
        c_w2 = cp(w2_hbm, w2_v, 0, F, 0, D, b + 4)
        kcp[0].start(); xcp[0].start(); vcp[0].start()
        for g in range(1, NW):
            kcp[g].start(); vcp[g].start()
        for i in range(1, n1):
            xcp[i].start()
        c_wo.start(); c_q.start(); c_w1.start(); c_w3.start(); c_w2.start()

        kv_v[...] = jnp.zeros(kv_v.shape, f32)
        zacc_v[...] = jnp.zeros(zacc_v.shape, f32)

        def p1_body(xt, first=False):
            def kvproj(g):
                return dot(xt, wqkv_v[:, D + g*128:D + (g+1)*128]), dot(xt, wqkv_v[:, 2*D + g*128:2*D + (g+1)*128])
            def fin(g, k, v):
                pk = phi(k).astype(bf16)
                zacc_v[:, g*128:(g+1)*128] += jnp.sum(pk.astype(f32).reshape(TS1 // 8, 8, 128), axis=0)
                kv = jax.lax.dot_general(pk, v.astype(bf16), (((0,), (0,)), ((), ())), preferred_element_type=f32)
                kv_v[g] += kv
            prev = None
            for g in range(NG):
                if first and g > 0 and g % GW == 0:
                    kcp[g // GW].wait(); vcp[g // GW].wait()
                cur = kvproj(g)
                if prev is not None:
                    fin(g - 1, *prev)
                prev = cur
            fin(NG - 1, *prev)

        with sc("w0"):
            kcp[0].wait(); xcp[0].wait(); vcp[0].wait()
        with sc("p1a"):
            p1_body(x_v[0:TS1, :], True)
        def p1(i, _):
            cp(x_hbm, x_v, 0, TS1, 0, D, i).wait()
            p1_body(x_v[pl.ds(pl.multiple_of(i * TS1, TS1), TS1), :])
            return 0
        with sc("p1b"):
            jax.lax.fori_loop(1, n1, p1, 0)

        c_wo.wait()
        r = jax.lax.broadcasted_iota(jnp.int32, (128, 128), 0)
        c = jax.lax.broadcasted_iota(jnp.int32, (128, 128), 1)
        same = (r // DH) == (c // DH)
        for g in range(NG):
            kvg = jnp.where(same, kv_v[g], 0.0).astype(bf16)
            m_v[g*128:(g+1)*128, :] = dot(kvg, wo_v[g*128:(g+1)*128, :]).astype(bf16)
            zrow = jnp.sum(zacc_v[:, g*128:(g+1)*128], axis=0, keepdims=True)
            zb = jnp.broadcast_to(zrow, (128, 128)).T
            z_v[g] = jnp.where(same, zb, 0.0).astype(bf16)

        with sc("w1"):
            c_q.wait(); c_w1.wait(); c_w3.wait(); c_w2.wait()
        gw8 = gw_ref[...].astype(f32)
        gw = cat([gw8[g:g+1, :] for g in range(NG)])

        def ocp(slot, i):
            return pltpu.make_async_copy(o_v.at[slot], o_hbm.at[pl.ds(pl.multiple_of(i * TS2, TS2), TS2), :], osems.at[slot])

        def p2(i, _):
            slot = i % 2
            @pl.when(i >= 2)
            def _():
                ocp(slot, i - 2).wait()
            xt = x_v[pl.ds(pl.multiple_of(i * TS2, TS2), TS2), :]
            gate = sigmoid(jnp.sum(xt.astype(f32) * gw, axis=-1, keepdims=True))
            omg = 1.0 - gate
            def gu(j):
                return dot(xt, w1_v[:, j*FC:(j+1)*FC]), dot(xt, w3_v[:, j*FC:(j+1)*FC])
            def hh(gt, up):
                return ((gt * sigmoid(gt)) * (up * omg)).astype(bf16)
            def w2c(j):
                return w2_v[j*FC:(j+1)*FC, :]
            q = dot(xt, wqkv_v[:, 0:D])
            gu0 = gu(0)
            pq = phi(q)
            pqb = pq.astype(bf16)
            den = cat([dot(pqb[:, g*128:(g+1)*128], z_v[g]) for g in range(NG)]) + 1e-6
            gu1 = gu(1)
            pqn = (pq * (gate * rcp(den))).astype(bf16)
            acc = dot(hh(*gu0), w2c(0))
            prev = gu1
            for j in range(2, nf):
                cur = gu(j)
                acc = acc + dot(hh(*prev), w2c(j - 1))
                prev = cur
            acc = acc + dot(pqn, m_v[...])
            acc = acc + dot(hh(*prev), w2c(nf - 1))
            o_v[slot] = acc.astype(bf16)
            ocp(slot, i).start()
            return 0
        with sc("p2"):
            jax.lax.fori_loop(0, n2, p2, 0)
        with sc("wend"):
            ocp((n2 - 2) % 2, n2 - 2).wait()
            ocp((n2 - 1) % 2, n2 - 1).wait()

    @jax.jit
    def fn(A_x, A_wqkv, A_wo, B_x, B_w1, B_w3, B_w2, gate_w):
        x2 = A_x.reshape(S, D)
        gw = gate_w.reshape(NG, 128)
        any_ = pl.BlockSpec(memory_space=pl.ANY)
        out = pl.pallas_call(
            kern,
            in_specs=[any_] * 6 + [pl.BlockSpec(memory_space=pltpu.VMEM)],
            out_specs=any_,
            out_shape=jax.ShapeDtypeStruct((S, D), bf16),
            scratch_shapes=[
                pltpu.VMEM((S, D), bf16), pltpu.VMEM((D, 3 * D), bf16), pltpu.VMEM((D, D), bf16),
                pltpu.VMEM((D, F), bf16), pltpu.VMEM((D, F), bf16), pltpu.VMEM((F, D), bf16),
                pltpu.VMEM((D, D), bf16), pltpu.VMEM((NG, 128, 128), bf16), pltpu.VMEM((NG, 128, 128), f32),
                pltpu.VMEM((8, D), f32), pltpu.VMEM((2, TS2, D), bf16),
                pltpu.SemaphoreType.DMA((n1 + 2 * NG + 5,)), pltpu.SemaphoreType.DMA((2,)),
            ],
            compiler_params=pltpu.CompilerParams(vmem_limit_bytes=100 * 1024 * 1024),
        )(x2, A_wqkv, A_wo, B_w1, B_w3, B_w2, gw)
        return out.reshape(1, S, D)
    return fn


_impl = make(GW=2)

@jax.jit
def pallas_gated_mix__linear_attn_block__glu_gated_swiglu__prompt_kernel(A_x, A_wqkv, A_wo, B_x, B_w1, B_w3, B_w2, gate_w):
    return _impl(A_x, A_wqkv, A_wo, B_x, B_w1, B_w3, B_w2, gate_w)
```

```python
import functools
import contextlib
import jax
import jax.numpy as jnp
import jax.experimental.pallas as pl
import jax.experimental.pallas.tpu as pltpu

S, D, F, H = 2048, 1024, 3584, 32
DH = D // H
bf16, f32, u32 = jnp.bfloat16, jnp.float32, jnp.uint32
NG = D // 128
D2 = D // 2
F2 = F // 2
F4 = F // 4
Q4 = D // 4
TS1 = 512
N1 = S // TS1
NT = S // 256

def phi(t):
    return jnp.where(t > 0, t + 1.0, jnp.exp(t)) + 1e-6

def rcp(y):
    return pltpu.reciprocal(y, approx=True)

def sigmoid(x):
    return rcp(1.0 + jnp.exp(-x))

def dot(a, b):
    return jnp.dot(a, b, preferred_element_type=f32)

def cat(xs, axis=1):
    return xs[0] if len(xs) == 1 else jnp.concatenate(xs, axis=axis)

def a_combos(a11, a12, a21, a22):
    return [(a11 + a22).astype(bf16), (a21 + a22).astype(bf16), a11.astype(bf16), a22.astype(bf16),
            (a11 + a12).astype(bf16), (a21 - a11).astype(bf16), (a12 - a22).astype(bf16)]

def b_combos(b11, b12, b21, b22):
    return [b11 + b22, b11, b12 - b22, b21 - b11, b22, b11 + b12, b21 + b22]

def c_combos(m):
    m1, m2, m3, m4, m5, m6, m7 = m
    return ((m1 + m4) - m5) + m7, m3 + m5, m2 + m4, ((m1 - m2) + m3) + m6

def make(scopes=False, RC=8, CW=256, w0groups=((0, 1), (1, 3), (3, 8)), split=(0.5, 0.5), st_from=1):
    sc = (lambda n: jax.named_scope(n)) if scopes else (lambda n: contextlib.nullcontext())
    NW = len(w0groups)
    def kern(x_hbm, wqkv_hbm, wo_hbm, w1_hbm, w3_hbm, w2_hbm, gw_hbm, o_hbm,
             x_v, tk_v, tv_v, wo_v, tq_v, t1_v, t3_v, r_v, xs_v, sq_v, g_v, omg_v, macc_v, z_v, kv_v, zacc_v, gw_v, o_v, sems, osems):
        sem_next = [0]
        def new_sem():
            sem_next[0] += 1
            return sems.at[sem_next[0] - 1]
        dma = pltpu.make_async_copy
        ds = pl.ds
        xcp = [[dma(x_hbm.at[ds(i * TS1, TS1), :], x_v.at[ds(i * TS1, TS1), :], new_sem())] for i in range(N1)]
        ORDER = (0, 4, 1, 5, 2, 6, 3, 7)
        kvcp = []
        for (a0, a1) in w0groups:
            s = new_sem(); cs = []
            for pos in range(a0, a1):
                g = ORDER[pos]; side, p = divmod(g, 4)
                for c0, t_ref in ((D, tk_v), (2 * D, tv_v)):
                    for qr, slot in ((0, (1, 7)[side]), (1, (8, 4)[side])):
                        cs.append(dma(wqkv_hbm.at[ds(qr * D2, D2), ds(c0 + g * 128, 128)], t_ref.at[slot, :, ds(p * 128, 128)], s))
            kvcp.append(cs)
        QUADS = ((1, 0, 0), (2, 0, 1), (3, 1, 0), (4, 1, 1))
        def quad1(src, dst, c0, ch, w, hf):
            s = new_sem()
            return [dma(src.at[ds(qr * D2, D2), ds(c0 + qc * ch + hf * w, w)], dst.at[slot, hf], s) for slot, qr, qc in QUADS]
        def quad2(hf):
            s = new_sem()
            return [dma(w2_hbm.at[ds(qr * F2 + hf * F4, F4), ds(qc * D2, D2)], r_v.at[slot, hf, ds(Q4, F4), :], s) for slot, qr, qc in QUADS]
        cq = [quad1(wqkv_hbm, tq_v, 0, D2, Q4, hf) for hf in range(2)]
        c1 = [quad1(w1_hbm, t1_v, 0, F2, F4, hf) for hf in range(2)]
        c3 = [quad1(w3_hbm, t3_v, 0, F2, F4, hf) for hf in range(2)]
        c2 = [quad2(hf) for hf in range(2)]
        cwo = [dma(wo_hbm, wo_v, new_sem())]
        cgw = [dma(gw_hbm, gw_v, new_sem())]
        def start(*css):
            for cs in css:
                for c in cs: c.start()
        def wait(*css):
            for cs in css:
                for c in cs: c.wait()
        start(kvcp[0][:2], xcp[0], kvcp[0][2:], *kvcp[1:])
        start(xcp[1], cgw, cq[0], cq[1], xcp[2], xcp[3], c1[0], c1[1], c3[0], c3[1], cwo, c2[0], c2[1])

        kv_v[...] = jnp.zeros(kv_v.shape, f32)
        zacc_v[...] = jnp.zeros(zacc_v.shape, f32)

        zm = []
        def gate_(v, tk):
            u = pltpu.bitcast(v, u32)
            z = pltpu.bitcast(tk, u32) & zm[0]
            u = u | jnp.tile(z[0:min(8, u.shape[0])], (max(1, u.shape[0] // 8), u.shape[1] // 128))
            return pltpu.bitcast(u, bf16).astype(f32)

        def prep_task(t_ref, hf, r0, nr, c0, nc):
            def run(tk):
                rows = ds(r0, nr); cols = ds(c0, nc)
                s12, s21 = (2, 3) if hf is not None else (7, 8)
                ix = (lambda slot: (slot, hf, rows, cols)) if hf is not None else (lambda slot: (slot, rows, cols))
                b11 = gate_(t_ref[ix(1)], tk); b12 = gate_(t_ref[ix(s12)], tk)
                b21 = gate_(t_ref[ix(s21)], tk); b22 = gate_(t_ref[ix(4)], tk)
                t_ref[ix(0)] = (b11 + b22).astype(bf16)
                t_ref[ix(2)] = (b12 - b22).astype(bf16)
                t_ref[ix(3)] = (b21 - b11).astype(bf16)
                t_ref[ix(5)] = (b11 + b12).astype(bf16)
                t_ref[ix(6)] = (b21 + b22).astype(bf16)
            return run
        def prep_tasks(t_ref, hf, r0, nrows):
            W = t_ref.shape[-1]
            return [prep_task(t_ref, hf, r0 + r, RC, c0, min(CW, W - c0)) for r in range(0, nrows, RC) for c0 in range(0, W, CW)]
        def xs_task(i, r0, nr, c0, nc):
            def run(tk):
                a11 = gate_(x_v[ds(i * 256 + r0, nr), ds(c0, nc)], tk); a12 = gate_(x_v[ds(i * 256 + r0, nr), ds(D2 + c0, nc)], tk)
                a21 = gate_(x_v[ds(i * 256 + 128 + r0, nr), ds(c0, nc)], tk); a22 = gate_(x_v[ds(i * 256 + 128 + r0, nr), ds(D2 + c0, nc)], tk)
                for j, s_ in enumerate(a_combos(a11, a12, a21, a22)):
                    xs_v[i, j, ds(r0, nr), ds(c0, nc)] = s_
            return run
        def xs_tasks(t1):
            return [xs_task(2 * t1 + i, r0, RC, c0, CW) for i in range(2) for r0 in range(0, 128, RC) for c0 in range(0, D2, CW)]
        gwl = []
        def gate_task(r0):
            def run(tk):
                rows = ds(r0, 16)
                tot = None
                for g in range(NG):
                    t_ = gate_(x_v[rows, g*128:(g+1)*128], tk) * gwl[0][g:g+1, :]
                    tot = t_ if tot is None else tot + t_
                gt = jnp.broadcast_to(sigmoid(jnp.sum(tot, axis=-1, keepdims=True)), (16, 128))
                g_v[rows, :] = gt
                omg_v[rows, :] = 1.0 - gt
            return run
        def gate_tasks(t1):
            return [gate_task(t1 * TS1 + r) for r in range(0, TS1, 16)]
        TK = prep_tasks(tk_v, None, 0, D2); TV = prep_tasks(tv_v, None, 0, D2)
        TQ = prep_tasks(tq_v, 0, 0, D2) + prep_tasks(tq_v, 1, 0, D2)
        T1 = [prep_tasks(t1_v, hf, 0, D2) for hf in range(2)]
        T3 = [prep_tasks(t3_v, hf, 0, D2) for hf in range(2)]
        T2 = [prep_tasks(r_v, hf, Q4, F4) for hf in range(2)]

        def spread(tasks, slots):
            out = {g: [] for g in slots}
            for n, t in enumerate(tasks):
                out[slots[n * len(slots) // len(tasks)]].append(t)
            return out
        def run_tasks(tl, results):
            ticks = [r[a:a + 8, :] for r in results for a in range(0, r.shape[0], 8)]
            for n_, task in enumerate(tl):
                task(ticks[n_ * len(ticks) // len(tl)])

        def fin(g, k, v):
            pk = phi(k).astype(bf16)
            zacc_v[:, g*128:(g+1)*128] += jnp.sum(pk.astype(f32).reshape(TS1 // 8, 8, 128), axis=0)
            kv_v[g] += jax.lax.dot_general(pk, v.astype(bf16), (((0,), (0,)), ((), ())), preferred_element_type=f32)
        def p1_tile(t, waits, tasks):
            xt = x_v[t * TS1:(t + 1) * TS1, :]
            def kvproj(g):
                side, p = divmod(g, 4)
                top, bot = ((1, 8), (7, 4))[side]
                cs = slice(p * 128, (p + 1) * 128)
                return (dot(xt, cat([tk_v[top, :, cs], tk_v[bot, :, cs]], 0)), dot(xt, cat([tv_v[top, :, cs], tv_v[bot, :, cs]], 0)))
            prev = None
            for pos in range(NG):
                if pos in waits:
                    wait(*waits[pos])
                g = ORDER[pos]
                cur = kvproj(g)
                run_tasks(tasks.get(pos, ()), cur)
                if prev is not None:
                    fin(*prev)
                prev = (g,) + cur
            fin(*prev)
        def p1_tile_st(t, tasks):
            xs = [[xs_v[2 * t + i, j] for j in range(7)] for i in range(2)]
            def proj(t_ref, p, tl):
                ms = [[dot(xs[i][j], t_ref[j, :, p*128:(p+1)*128]) for j in range(7)] for i in range(2)]
                run_tasks(tl, ms[0] + ms[1])
                c = [c_combos(m) for m in ms]
                return (cat([c[0][0], c[0][2], c[1][0], c[1][2]], 0), cat([c[0][1], c[0][3], c[1][1], c[1][3]], 0))
            prev = None
            for p in range(4):
                kk = proj(tk_v, p, tasks.get(2 * p, ()))
                if prev is not None:
                    fin(prev[0], prev[1][0], prev[2][0])
                vv = proj(tv_v, p, tasks.get(2 * p + 1, ()))
                if prev is not None:
                    fin(prev[0] + 4, prev[1][1], prev[2][1])
                prev = (p, kk, vv)
            fin(prev[0], prev[1][0], prev[2][0]); fin(prev[0] + 4, prev[1][1], prev[2][1])

        with sc("w0"):
            wait(kvcp[0], xcp[0])
        zm.append((pltpu.bitcast(x_v[0:16, 0:128], u32) >> 31) >> 1)
        n1a = int(len(T1[1]) * split[0]); n3a = int(len(T3[1]) * split[1])
        W0 = {w0groups[n][0]: [kvcp[n]] for n in range(1, NW)}
        last0 = w0groups[-1][0]
        with sc("p1_0"):
            W0[last0 + 2] = [xcp[1]]
            tk0 = spread(TK + TV, list(range(last0, last0 + 3)))
            tk0.update(spread(xs_tasks(1), list(range(last0 + 3, NG))))
            p1_tile(0, W0, tk0)
        with sc("p1_1"):
            wait(cgw, cq[0], cq[1], xcp[2])
            gwl.append(gw_v[...].astype(f32))
            p1_tile_st(1, spread(xs_tasks(2) + xs_tasks(0) + gate_tasks(0) + gate_tasks(1) + TQ, list(range(8))))
        with sc("p1_2"):
            wait(xcp[3], c1[0], c1[1])
            p1_tile_st(2, spread(xs_tasks(3) + gate_tasks(2) + T1[0] + T1[1][:n1a], list(range(8))))
        with sc("p1_3"):
            wait(c3[0], c3[1])
            p1_tile_st(3, spread(gate_tasks(3) + T1[1][n1a:] + T3[0] + T3[1][:n3a], list(range(8))))

        with sc("mph"):
            wait(cwo)
            r = jax.lax.broadcasted_iota(jnp.int32, (128, 128), 0)
            c = jax.lax.broadcasted_iota(jnp.int32, (128, 128), 1)
            same = (r // DH) == (c // DH)
            def mblk(g):
                kvg = jnp.where(same, kv_v[g], 0.0).astype(bf16)
                return dot(kvg, wo_v[g*128:(g+1)*128, :])
            for g in range(NG):
                zrow = jnp.sum(zacc_v[:, g*128:(g+1)*128], axis=0, keepdims=True)
                zb = jnp.broadcast_to(zrow, (128, 128)).T
                z_v[g] = jnp.where(same, zb, 0.0).astype(bf16)
            for p in range(4):
                mt = mblk(p); mb = mblk(p + 4)
                tb = b_combos(mt[:, :D2], mt[:, D2:], mb[:, :D2], mb[:, D2:])
                for j in range(7):
                    r_v[j, p // 2, ds((p % 2) * 128, 128), :] = tb[j].astype(bf16)

        with sc("p1b"):
            NJ = NT * 4
            NJ0 = 6
            lt = spread(T3[1][n3a:], list(range(NJ0)))
            lt.update(spread(T2[0] + T2[1], list(range(NJ0, NJ))))
            def qjob(n):
                i, p = divmod(n, 4)
                ms = [dot(xs_v[i, j], tq_v[j, p // 2, :, (p % 2) * 128:(p % 2 + 1) * 128]) for j in range(7)]
                run_tasks(lt.get(n, ()), ms)
                return c_combos(ms)
            def denjob(n, q4):
                i, p = divmod(n, 4)
                out = []
                for k, q in enumerate(q4):
                    pq = phi(q)
                    out.append((pq, dot(pq.astype(bf16), z_v[p + 4 * (k % 2)]) + 1e-6))
                return out
            def norm(n, pd):
                i, p = divmod(n, 4)
                gts = (g_v[i * 256:i * 256 + 128, :], g_v[i * 256 + 128:(i + 1) * 256, :])
                ss = a_combos(*[pq * (gts[k // 2] * rcp(den)) for k, (pq, den) in enumerate(pd)])
                for j in range(7):
                    sq_v[i, p // 2, j, :, (p % 2) * 128:(p % 2 + 1) * 128] = ss[j]
            q_prev = None; pd_prev = None
            for n in range(NJ + 2):
                if n == NJ0:
                    wait(c2[0], c2[1])
                q_cur = qjob(n) if n < NJ else None
                pd_cur = denjob(n - 1, q_prev) if 1 <= n <= NJ else None
                if n >= 2:
                    norm(n - 2, pd_prev)
                q_prev, pd_prev = q_cur, pd_cur

        def ocp(slot, i):
            return dma(o_v.at[slot], o_hbm.at[ds(pl.multiple_of(i * 256, 256), 256), :], osems.at[slot])

        def p2(t, _):
            i = t // 2
            hf = t % 2
            slot = i % 2
            @pl.when(jnp.logical_and(hf == 0, i >= 2))
            def _():
                ocp(slot, i - 2).wait()
            r0 = pl.multiple_of(i * 256, 256)
            oms = (omg_v[ds(r0, 128), :], omg_v[ds(r0 + 128, 128), :])
            xs = [xs_v[i, j] for j in range(7)]
            first = hf == 0

            def f1(t_ref, pp):
                return c_combos([dot(xs[j], t_ref[j, hf, :, pp*128:(pp+1)*128]) for j in range(7)])
            def gujob(pp):
                return f1(t1_v, pp), f1(t3_v, pp)
            def gufin(gu):
                g4, u4 = gu
                return a_combos(*[(g4[k] * sigmoid(g4[k])) * (u4[k] * oms[k // 2]) for k in range(4)])

            gu = [None] * 7; sh = [None] * 7
            gu[0] = gujob(0)
            gu[1] = gujob(1); sh[0] = gufin(gu[0])
            gu[2] = gujob(2); sh[1] = gufin(gu[1])
            for j in range(7):
                d = dot(cat([sq_v[i, hf, j], sh[0][j], sh[1][j]]), r_v[j, hf, 0:512, :])
                macc_v[j] = jnp.where(first, 0.0, macc_v[j]) + d
            gu[3] = gujob(3); sh[2] = gufin(gu[2])
            gu[4] = gujob(4); sh[3] = gufin(gu[3])
            gu[5] = gujob(5); sh[4] = gufin(gu[4])
            gu[6] = gujob(6); sh[5] = gufin(gu[5])
            for j in range(7):
                macc_v[j] += dot(cat([sh[2][j], sh[3][j], sh[4][j], sh[5][j]]), r_v[j, hf, 512:1024, :])
            sh[6] = gufin(gu[6])
            for n in range(4):
                cs = slice(n * 128, (n + 1) * 128)
                ms = []
                for j in range(7):
                    mj = macc_v[j, :, cs] + dot(sh[6][j], r_v[j, hf, 1024:1152, cs])
                    macc_v[j, :, cs] = mj
                    ms.append(mj)
                c11, c12, c21, c22 = c_combos(ms)
                o_v[slot, 0:128, n*128:(n+1)*128] = c11.astype(bf16)
                o_v[slot, 0:128, D2 + n*128:D2 + (n+1)*128] = c12.astype(bf16)
                o_v[slot, 128:256, n*128:(n+1)*128] = c21.astype(bf16)
                o_v[slot, 128:256, D2 + n*128:D2 + (n+1)*128] = c22.astype(bf16)
            @pl.when(hf == 1)
            def _():
                ocp(slot, i).start()
            return 0
        with sc("p2"):
            jax.lax.fori_loop(0, 2 * NT, p2, 0)
        with sc("wend"):
            ocp((NT - 2) % 2, NT - 2).wait()
            ocp((NT - 1) % 2, NT - 1).wait()

    @jax.jit
    def fn(A_x, A_wqkv, A_wo, B_x, B_w1, B_w3, B_w2, gate_w):
        x2 = A_x.reshape(S, D)
        gw = gate_w.reshape(NG, 128)
        any_ = pl.BlockSpec(memory_space=pl.ANY)
        V = pltpu.VMEM
        out = pl.pallas_call(
            kern,
            in_specs=[any_] * 7,
            out_specs=any_,
            out_shape=jax.ShapeDtypeStruct((S, D), bf16),
            scratch_shapes=[
                V((S, D), bf16), V((9, D2, D2), bf16), V((9, D2, D2), bf16), V((D, D), bf16),
                V((7, 2, D2, Q4), bf16), V((7, 2, D2, F4), bf16), V((7, 2, D2, F4), bf16), V((7, 2, Q4 + F4, D2), bf16),
                V((NT, 7, 128, D2), bf16), V((NT, 2, 7, 128, Q4), bf16), V((S, 128), f32), V((S, 128), f32), V((7, 128, D2), f32),
                V((NG, 128, 128), bf16), V((NG, 128, 128), f32),
                V((8, D), f32), V((NG, 128), bf16), V((2, 256, D), bf16),
                pltpu.SemaphoreType.DMA((N1 + NW + 10,)), pltpu.SemaphoreType.DMA((2,)),
            ],
            compiler_params=pltpu.CompilerParams(vmem_limit_bytes=110 * 1024 * 1024),
        )(x2, A_wqkv, A_wo, B_w1, B_w3, B_w2, gw)
        return out.reshape(1, S, D)
    return fn


_impl = make()

@jax.jit
def pallas_gated_mix__linear_attn_block__glu_gated_swiglu__prompt_kernel(A_x, A_wqkv, A_wo, B_x, B_w1, B_w3, B_w2, gate_w):
    return _impl(A_x, A_wqkv, A_wo, B_x, B_w1, B_w3, B_w2, gate_w)
```

```python
import functools
import contextlib
import jax
import jax.numpy as jnp
import jax.experimental.pallas as pl
import jax.experimental.pallas.tpu as pltpu

S, D, F, H = 2048, 1024, 3584, 32
DH = D // H
bf16, f32, u32 = jnp.bfloat16, jnp.float32, jnp.uint32
NG = D // 128
D2 = D // 2
D4 = D // 4
F4 = F // 4
TS1 = 512
N1 = S // TS1
NT = S // 256

def phi(t):
    return jnp.where(t > 0, t + 1.0, jnp.exp(t)) + 1e-6

def rcp(y):
    return pltpu.reciprocal(y, approx=True)

def sigmoid(x):
    return rcp(1.0 + jnp.exp(-x))

def dot(a, b):
    return jnp.dot(a, b, preferred_element_type=f32)

def cat(xs, axis=1):
    return xs[0] if len(xs) == 1 else jnp.concatenate(xs, axis=axis)

def a_combos(a11, a12, a21, a22):
    return [a11 + a22, a21 + a22, a11, a22, a11 + a12, a21 - a11, a12 - a22]

def b_combos(b11, b12, b21, b22):
    return [b11 + b22, b11, b12 - b22, b21 - b11, b22, b11 + b12, b21 + b22]

def c_combos(m):
    m1, m2, m3, m4, m5, m6, m7 = m
    return ((m1 + m4) - m5) + m7, m3 + m5, m2 + m4, ((m1 - m2) + m3) + m6

def combos2(fn, blk):
    lvl1 = {(r, c): fn(blk[r, c], blk[r, 2 + c], blk[2 + r, c], blk[2 + r, 2 + c]) for r in range(2) for c in range(2)}
    out = []
    for i in range(7):
        out += fn(lvl1[0, 0][i], lvl1[0, 1][i], lvl1[1, 0][i], lvl1[1, 1][i])
    return out

def c_combos2(ms):
    inner = [c_combos(ms[7 * i:7 * i + 7]) for i in range(7)]
    out = {}
    for q, (r, c) in enumerate(((0, 0), (0, 1), (1, 0), (1, 1))):
        c11, c12, c21, c22 = c_combos([inner[i][q] for i in range(7)])
        out[r, c] = c11; out[r, 2 + c] = c12; out[2 + r, c] = c21; out[2 + r, 2 + c] = c22
    return out

RAW = {(0, 0): 8, (1, 1): 11, (2, 2): 29, (3, 3): 32}
for _n, _k in enumerate([(0, 1), (1, 0), (0, 2), (0, 3), (1, 2), (1, 3)]):
    RAW[_k] = 35 + _n
for _n, _k in enumerate([(2, 0), (2, 1), (3, 0), (3, 1), (2, 3), (3, 2)]):
    RAW[_k] = 42 + _n
BQ = {0: ((0, 0), (1, 1), 1), 1: ((0, 0),), 2: ((0, 1), (1, 1), -1), 3: ((1, 0), (0, 0), -1), 4: ((1, 1),),
      5: ((0, 0), (0, 1), 1), 6: ((1, 0), (1, 1), 1)}

def make(scopes=False, RC=8, CW=256, w0groups=((0, 1), (1, 3), (3, 8)), nj0=4):
    sc = lambda n: jax.named_scope(n) if (scopes is True or (scopes and n in scopes)) else contextlib.nullcontext()
    NW = len(w0groups)
    def kern(x_hbm, wqkv_hbm, wo_hbm, w1_hbm, w3_hbm, w2_hbm, gw_hbm, o_hbm,
             x_v, tk_v, tv_v, wo_v, tq_v, tm_v, t1_v, t3_v, t2_v, xs_v, a_v, g_v, omg_v, macc_v, z_v, kv_v, zacc_v, gw_v, o_v,
             sems, osems):
        sem_next = [0]
        def new_sem():
            sem_next[0] += 1
            return sems.at[sem_next[0] - 1]
        dma = pltpu.make_async_copy
        ds = pl.ds
        xcp = [[dma(x_hbm.at[ds(i * TS1, TS1), :], x_v.at[ds(i * TS1, TS1), :], new_sem())] for i in range(N1)]
        ORDER = (0, 4, 1, 5, 2, 6, 3, 7)
        kvcp = []
        for (a0, a1) in w0groups:
            s = new_sem(); cs = []
            for pos in range(a0, a1):
                g = ORDER[pos]; side, p = divmod(g, 4)
                for c0, t_ref in ((D, tk_v), (2 * D, tv_v)):
                    for qr, slot in ((0, (1, 7)[side]), (1, (8, 4)[side])):
                        cs.append(dma(wqkv_hbm.at[ds(qr * D2, D2), ds(c0 + g * 128, 128)], t_ref.at[slot, :, ds(p * 128, 128)], s))
            kvcp.append(cs)
        s_ = new_sem()
        cq = [dma(wqkv_hbm.at[ds(qr * D2, D2), ds(qc * D2, D2)], tq_v.at[slot], s_) for slot, qr, qc in ((1, 0, 0), (2, 0, 1), (3, 1, 0), (4, 1, 1))]
        def blocks(src, dst, kb, nb, part):
            s = new_sem(); hr = kb // 2
            return [dma(src.at[ds(kq * kb + part * hr, hr), ds(nq * nb, nb)], dst.at[slot, ds(part * hr, hr), :], s)
                    for (kq, nq), slot in RAW.items()]
        c1 = [blocks(w1_hbm, t1_v, D4, F4, part) for part in range(2)]
        c3 = [blocks(w3_hbm, t3_v, D4, F4, part) for part in range(2)]
        c2 = [blocks(w2_hbm, t2_v, F4, D4, part) for part in range(2)]
        cwo = [dma(wo_hbm, wo_v, new_sem())]
        cgw = [dma(gw_hbm, gw_v, new_sem())]
        def start(*css):
            for cs in css:
                for c in cs: c.start()
        def wait(*css):
            for cs in css:
                for c in cs: c.wait()
        start(kvcp[0][:2], xcp[0], kvcp[0][2:], *kvcp[1:])
        start(xcp[1], cgw, cq, xcp[2], xcp[3])

        kv_v[...] = jnp.zeros(kv_v.shape, f32)
        zacc_v[...] = jnp.zeros(zacc_v.shape, f32)

        zm = []
        def gate_(v, tk):
            u = pltpu.bitcast(v, u32)
            z = pltpu.bitcast(tk, u32) & zm[0]
            u = u | jnp.tile(z[0:min(8, u.shape[0])], (max(1, u.shape[0] // 8), u.shape[1] // 128))
            return pltpu.bitcast(u, bf16).astype(f32)

        def pieces(t_ref, r0, nrows):
            W = t_ref.shape[-1]; full = W // CW * CW
            out = [(r0 + r, RC, c0, CW) for r in range(0, nrows, RC) for c0 in range(0, full, CW)]
            if full < W:
                out += [(r0 + r, 2 * RC, full, W - full) for r in range(0, nrows, 2 * RC)]
            return out
        def prep1_task(t_ref, s12, s21, piece):
            r0, nr, c0, nc = piece
            def run(tk):
                ix = lambda slot: (slot, ds(r0, nr), ds(c0, nc))
                tb = b_combos(gate_(t_ref[ix(1)], tk), gate_(t_ref[ix(s12)], tk), gate_(t_ref[ix(s21)], tk), gate_(t_ref[ix(4)], tk))
                for j in (0, 2, 3, 5, 6):
                    t_ref[ix(j)] = tb[j].astype(bf16)
            return run
        def prep2_task(t_ref, r0, c0, i):
            def run(tk):
                ix = lambda slot: (slot, ds(r0, 8), ds(c0, 128))
                q = BQ[i]; l1 = []
                for r in range(2):
                    for c in range(2):
                        a = gate_(t_ref[ix(RAW[2 * q[0][0] + r, 2 * q[0][1] + c])], tk)
                        if len(q) == 3:
                            b = t_ref[ix(RAW[2 * q[1][0] + r, 2 * q[1][1] + c])].astype(f32)
                            a = a + b if q[2] > 0 else a - b
                        l1.append(a)
                for j, v in enumerate(b_combos(*l1)):
                    if i in (1, 4) and j in (1, 4):
                        continue
                    t_ref[ix(7 * i + j)] = v.astype(bf16)
            return run
        def prep2_tasks(t_ref, r0, nrows):
            return [prep2_task(t_ref, r0 + r, c0, i) for r in range(0, nrows, 8) for c0 in range(0, t_ref.shape[-1], 128) for i in range(7)]
        def xs_task(i, r0, c0):
            def run(tk):
                def ld(rr, cc): return gate_(x_v[ds(i * 256 + rr + r0, RC), ds(cc + c0, CW)], tk)
                for j, s_ in enumerate(a_combos(ld(0, 0), ld(0, D2), ld(128, 0), ld(128, D2))):
                    xs_v[i, j, ds(r0, RC), ds(c0, CW)] = s_.astype(bf16)
            return run
        def xs_tasks(t1):
            return [xs_task(2 * t1 + i, r0, c0) for i in range(2) for r0 in range(0, 128, RC) for c0 in range(0, D2, CW)]
        gwl = []
        def gate_task(r0):
            def run(tk):
                rows = ds(r0, 16)
                tot = None
                for g in range(NG):
                    t_ = gate_(x_v[rows, g*128:(g+1)*128], tk) * gwl[0][g:g+1, :]
                    tot = t_ if tot is None else tot + t_
                gt = jnp.broadcast_to(sigmoid(jnp.sum(tot, axis=-1, keepdims=True)), (16, 128))
                g_v[rows, :] = gt
                omg_v[rows, :] = 1.0 - gt
            return run
        def gate_tasks(t1):
            return [gate_task(t1 * TS1 + r) for r in range(0, TS1, 16)]
        TK = [prep1_task(tk_v, 7, 8, p) for p in pieces(tk_v, 0, D2)]
        TV = [prep1_task(tv_v, 7, 8, p) for p in pieces(tv_v, 0, D2)]
        TQ = [prep1_task(tq_v, 2, 3, p) for p in pieces(tq_v, 0, D2)]
        T1 = [prep2_tasks(t1_v, part * 128, 128) for part in range(2)]
        T3 = [prep2_tasks(t3_v, part * 128, 128) for part in range(2)]
        T2 = [prep2_tasks(t2_v, part * 448, 448) for part in range(2)]

        def spread(tasks, slots):
            out = {g: [] for g in slots}
            for n, t in enumerate(tasks):
                out[slots[n * len(slots) // len(tasks)]].append(t)
            return out
        def mix(*lists):
            tagged = [((n + 0.5) / len(l), k, t) for k, l in enumerate(lists) for n, t in enumerate(l)]
            return [t for _, _, t in sorted(tagged, key=lambda e: e[:2])]
        def run_tasks(tl, results):
            if not tl:
                return
            ticks = [r[a:a + 8, c:c + 128] for r in results for c in range(0, r.shape[1], 128) for a in range(0, r.shape[0], 8)]
            for n_, task in enumerate(tl):
                task(ticks[n_ * len(ticks) // len(tl)])

        def fin(g, k, v):
            pk = phi(k).astype(bf16)
            zacc_v[:, g*128:(g+1)*128] += jnp.sum(pk.astype(f32).reshape(TS1 // 8, 8, 128), axis=0)
            kv_v[g] += jax.lax.dot_general(pk, v.astype(bf16), (((0,), (0,)), ((), ())), preferred_element_type=f32)
        def p1_tile(t, waits, tasks):
            xt = x_v[t * TS1:(t + 1) * TS1, :]
            def kvproj(g):
                side, p = divmod(g, 4)
                top, bot = ((1, 8), (7, 4))[side]
                cs = slice(p * 128, (p + 1) * 128)
                return (dot(xt, cat([tk_v[top, :, cs], tk_v[bot, :, cs]], 0)), dot(xt, cat([tv_v[top, :, cs], tv_v[bot, :, cs]], 0)))
            prev = None
            for pos in range(NG):
                if pos in waits:
                    wait(*waits[pos])
                g = ORDER[pos]
                cur = kvproj(g)
                run_tasks(tasks.get(pos, ()), cur)
                if prev is not None:
                    fin(*prev)
                prev = (g,) + cur
            fin(*prev)
        def p1_tile_st(t, tasks):
            xs = [[xs_v[2 * t + i, j] for j in range(7)] for i in range(2)]
            def proj(t_ref, p, tl):
                ms = [[dot(xs[i][j], t_ref[j, :, p*128:(p+1)*128]) for j in range(7)] for i in range(2)]
                run_tasks(tl, ms[0] + ms[1])
                c = [c_combos(m) for m in ms]
                return (cat([c[0][0], c[0][2], c[1][0], c[1][2]], 0), cat([c[0][1], c[0][3], c[1][1], c[1][3]], 0))
            prev = None
            for p in range(4):
                kk = proj(tk_v, p, tasks.get(2 * p, ()))
                if prev is not None:
                    fin(prev[0], prev[1][0], prev[2][0])
                vv = proj(tv_v, p, tasks.get(2 * p + 1, ()))
                if prev is not None:
                    fin(prev[0] + 4, prev[1][1], prev[2][1])
                prev = (p, kk, vv)
            fin(prev[0], prev[1][0], prev[2][0]); fin(prev[0] + 4, prev[1][1], prev[2][1])

        with sc("w0"):
            wait(kvcp[0], xcp[0])
        zm.append((pltpu.bitcast(x_v[0:16, 0:128], u32) >> 31) >> 1)
        W0 = {w0groups[n][0]: [kvcp[n]] for n in range(1, NW)}
        last0 = w0groups[-1][0]
        J8 = list(range(8))
        with sc("p1_0"):
            W0[last0 + 2] = [xcp[1]]
            tk0 = spread(TK + TV, list(range(last0, last0 + 3)))
            tk0.update(spread(xs_tasks(1), list(range(last0 + 3, NG))))
            start(c1[0], c1[1])
            p1_tile(0, W0, tk0)
        with sc("p1_1"):
            wait(cgw, cq, xcp[2])
            start(c3[0], c3[1], cwo)
            gwl.append(gw_v[...].astype(f32))
            p1_tile_st(1, spread(mix(xs_tasks(2), xs_tasks(0), gate_tasks(0) + gate_tasks(1), TQ), J8))
        with sc("p1_2"):
            wait(xcp[3], c1[0], c1[1])
            start(c2[0], c2[1])
            p1_tile_st(2, spread(mix(xs_tasks(3), gate_tasks(2), T1[0]), J8))
        with sc("p1_3"):
            p1_tile_st(3, spread(mix(gate_tasks(3), T1[1]), J8))

        with sc("mph"):
            wait(cwo, c3[0], c3[1])
            r = jax.lax.broadcasted_iota(jnp.int32, (128, 128), 0)
            c = jax.lax.broadcasted_iota(jnp.int32, (128, 128), 1)
            same = (r // DH) == (c // DH)
            def mblk(g):
                kvg = jnp.where(same, kv_v[g], 0.0).astype(bf16)
                return dot(kvg, wo_v[g*128:(g+1)*128, :])
            for g in range(NG):
                zrow = jnp.sum(zacc_v[:, g*128:(g+1)*128], axis=0, keepdims=True)
                zb = jnp.broadcast_to(zrow, (128, 128)).T
                z_v[g] = jnp.where(same, zb, 0.0).astype(bf16)
            for p in range(4):
                mt = mblk(p); mb = mblk(p + 4)
                for j, tb in enumerate(b_combos(mt[:, :D2], mt[:, D2:], mb[:, :D2], mb[:, D2:])):
                    tm_v[j, p * 128:(p + 1) * 128, :] = tb.astype(bf16)

        with sc("p1b"):
            NS = NT * 8
            lt = spread(T3[0] + T3[1], list(range(NS // 2)))
            lt.update(spread(T2[0] + T2[1], list(range(NS // 2, NS))))
            slot_no = [0]
            def tasks_next(ms):
                run_tasks(lt.get(slot_no[0], ()), ms)
                slot_no[0] += 1
                if slot_no[0] == NS // 2:
                    wait(c2[0], c2[1])
            def qjob(i, p):
                ms = [dot(xs_v[i, j], tq_v[j, :, p * 128:(p + 1) * 128]) for j in range(7)]
                tasks_next(ms)
                return c_combos(ms)
            def denjob(p, q4):
                out = []
                for k, q in enumerate(q4):
                    pq = phi(q)
                    out.append((pq, dot(pq.astype(bf16), z_v[p + 4 * (k % 2)]) + 1e-6))
                return out
            def norm(i, pd):
                gts = (g_v[i * 256:i * 256 + 128, :], g_v[i * 256 + 128:(i + 1) * 256, :])
                return [s.astype(bf16) for s in a_combos(*[pq * (gts[k // 2] * rcp(den)) for k, (pq, den) in enumerate(pd)])]
            def ajob(i, ss):
                lhs = [cat([ss[p][j] for p in range(4)]) for j in range(7)]
                for n in range(4):
                    cs = slice(n * 128, (n + 1) * 128)
                    ms = [dot(lhs[j], tm_v[j, :, cs]) for j in range(7)]
                    tasks_next(ms)
                    c11, c12, c21, c22 = c_combos(ms)
                    r0 = i * 256
                    a_v[r0:r0 + 128, n*128:(n+1)*128] = c11.astype(bf16)
                    a_v[r0:r0 + 128, D2 + n*128:D2 + (n+1)*128] = c12.astype(bf16)
                    a_v[r0 + 128:r0 + 256, n*128:(n+1)*128] = c21.astype(bf16)
                    a_v[r0 + 128:r0 + 256, D2 + n*128:D2 + (n+1)*128] = c22.astype(bf16)
            prev_q = None; prev_ss = None
            for i in range(NT):
                q = [None] * 4; ss = [None] * 4
                q[0] = qjob(i, 0)
                if i > 0:
                    prev_ss[3] = norm(i - 1, denjob(3, prev_q))
                q[1] = qjob(i, 1); pd0 = denjob(0, q[0])
                if i > 0:
                    ajob(i - 1, prev_ss)
                ss[0] = norm(i, pd0)
                q[2] = qjob(i, 2); ss[1] = norm(i, denjob(1, q[1]))
                q[3] = qjob(i, 3); ss[2] = norm(i, denjob(2, q[2]))
                prev_q, prev_ss = q[3], ss
            prev_ss[3] = norm(NT - 1, denjob(3, prev_q))
            ajob(NT - 1, prev_ss)

        def ocp(slot, i):
            return dma(o_v.at[slot], o_hbm.at[ds(pl.multiple_of(i * 256, 256), 256), :], osems.at[slot])

        def p2(i, _):
            slot = i % 2
            @pl.when(i >= 2)
            def _():
                ocp(slot, i - 2).wait()
            r0 = pl.multiple_of(i * 256, 256)
            oms = [omg_v[ds(r0 + rb * 64, 64), :] for rb in range(4)]
            xb = {(rb, kq): x_v[ds(r0 + rb * 64, 64), kq * D4:(kq + 1) * D4].astype(f32) for rb in range(4) for kq in range(4)}
            x2 = [v.astype(bf16) for v in combos2(a_combos, xb)]
            def f2(t_ref, p):
                return c_combos2([dot(x2[s], t_ref[s, :, p*128:(p+1)*128]) for s in range(49)])
            def gujob(p):
                return f2(t1_v, p), f2(t3_v, p)
            def gufin(gu):
                g, u = gu
                h = {k: (g[k] * sigmoid(g[k])) * (u[k] * oms[k[0]]) for k in g}
                return [s.astype(bf16) for s in combos2(a_combos, h)]
            gu = {}; sh = {}
            def l2(ps, first):
                for s in range(49):
                    d = dot(cat([sh[p][s] for p in ps]), t2_v[s, ps[0] * 128:(ps[-1] + 1) * 128, :])
                    macc_v[s] = d if first else macc_v[s] + d
            gu[0] = gujob(0)
            for p in (1, 2, 3, 4):
                gu[p] = gujob(p); sh[p - 1] = gufin(gu[p - 1])
            l2((0, 1, 2), True)
            for p in (5, 6):
                gu[p] = gujob(p); sh[p - 1] = gufin(gu[p - 1])
            l2((3, 4, 5), False)
            sh[6] = gufin(gu[6])
            for n in range(2):
                cs = slice(n * 128, (n + 1) * 128)
                ms = [macc_v[s, :, cs] + dot(sh[6][s], t2_v[s, 768:896, cs]) for s in range(49)]
                for (rb, nq), cblk in c_combos2(ms).items():
                    cols = slice(nq * D4 + n * 128, nq * D4 + (n + 1) * 128)
                    o_v[slot, rb * 64:(rb + 1) * 64, cols] = (cblk + a_v[ds(r0 + rb * 64, 64), cols].astype(f32)).astype(bf16)
            ocp(slot, i).start()
            return 0
        with sc("p2"):
            jax.lax.fori_loop(0, NT, p2, 0)
        with sc("wend"):
            ocp((NT - 2) % 2, NT - 2).wait()
            ocp((NT - 1) % 2, NT - 1).wait()

    @jax.jit
    def fn(A_x, A_wqkv, A_wo, B_x, B_w1, B_w3, B_w2, gate_w):
        x2 = A_x.reshape(S, D)
        gw = gate_w.reshape(NG, 128)
        any_ = pl.BlockSpec(memory_space=pl.ANY)
        V = pltpu.VMEM
        out = pl.pallas_call(
            kern,
            in_specs=[any_] * 7,
            out_specs=any_,
            out_shape=jax.ShapeDtypeStruct((S, D), bf16),
            scratch_shapes=[
                V((S, D), bf16), V((9, D2, D2), bf16), V((9, D2, D2), bf16), V((D, D), bf16),
                V((7, D2, D2), bf16), V((7, D2, D2), bf16),
                V((49, D4, F4), bf16), V((49, D4, F4), bf16), V((49, F4, D4), bf16),
                V((NT, 7, 128, D2), bf16), V((S, D), bf16), V((S, 128), f32), V((S, 128), f32),
                V((49, 64, D4), f32), V((NG, 128, 128), bf16), V((NG, 128, 128), f32),
                V((8, D), f32), V((NG, 128), bf16), V((2, 256, D), bf16),
                pltpu.SemaphoreType.DMA((N1 + NW + 9,)), pltpu.SemaphoreType.DMA((2,)),
            ],
            compiler_params=pltpu.CompilerParams(vmem_limit_bytes=126 * 1024 * 1024),
        )(x2, A_wqkv, A_wo, B_w1, B_w3, B_w2, gw)
        return out.reshape(1, S, D)
    return fn


_impl = make()

@jax.jit
def pallas_gated_mix__linear_attn_block__glu_gated_swiglu__prompt_kernel(A_x, A_wqkv, A_wo, B_x, B_w1, B_w3, B_w2, gate_w):
    return _impl(A_x, A_wqkv, A_wo, B_x, B_w1, B_w3, B_w2, gate_w)
```

```python
import jax
import jax.numpy as jnp
import jax.experimental.pallas as pl
import jax.experimental.pallas.tpu as pltpu

S, D, F, H = 2048, 1024, 3584, 32
DH = D // H
bf16, f32, u32 = jnp.bfloat16, jnp.float32, jnp.uint32
NG = D // 128
D2 = D // 2
D4 = D // 4
F4 = F // 4
TS1 = 512
N1 = S // TS1
NT = S // 256

def phi(t):
    return jnp.where(t > 0, t + 1.0, jnp.exp(t)) + 1e-6

def rcp(y):
    return pltpu.reciprocal(y, approx=True)

def sigmoid(x):
    return rcp(1.0 + jnp.exp(-x))

def dot(a, b):
    return jnp.dot(a, b, preferred_element_type=f32)

def cat(xs, axis=1):
    return xs[0] if len(xs) == 1 else jnp.concatenate(xs, axis=axis)

def a_combos(a11, a12, a21, a22):
    return [a11 + a22, a21 + a22, a11, a22, a11 + a12, a21 - a11, a12 - a22]

def b_combos(b11, b12, b21, b22):
    return [b11 + b22, b11, b12 - b22, b21 - b11, b22, b11 + b12, b21 + b22]

def c_combos(m):
    m1, m2, m3, m4, m5, m6, m7 = m
    return ((m1 + m4) - m5) + m7, m3 + m5, m2 + m4, ((m1 - m2) + m3) + m6

def combos2(fn, blk):
    lvl1 = {(r, c): fn(blk[r, c], blk[r, 2 + c], blk[2 + r, c], blk[2 + r, 2 + c]) for r in range(2) for c in range(2)}
    out = []
    for i in range(7):
        out += fn(lvl1[0, 0][i], lvl1[0, 1][i], lvl1[1, 0][i], lvl1[1, 1][i])
    return out

def c_combos2(ms):
    inner = [c_combos(ms[7 * i:7 * i + 7]) for i in range(7)]
    out = {}
    for q, (r, c) in enumerate(((0, 0), (0, 1), (1, 0), (1, 1))):
        c11, c12, c21, c22 = c_combos([inner[i][q] for i in range(7)])
        out[r, c] = c11; out[r, 2 + c] = c12; out[2 + r, c] = c21; out[2 + r, 2 + c] = c22
    return out

RAW = {(0, 0): 8, (1, 1): 11, (2, 2): 29, (3, 3): 32}
for _n, _k in enumerate([(0, 1), (1, 0), (0, 2), (0, 3), (1, 2), (1, 3)]):
    RAW[_k] = 35 + _n
for _n, _k in enumerate([(2, 0), (2, 1), (3, 0), (3, 1), (2, 3), (3, 2)]):
    RAW[_k] = 42 + _n
BQ = {0: ((0, 0), (1, 1), 1), 1: ((0, 0),), 2: ((0, 1), (1, 1), -1), 3: ((1, 0), (0, 0), -1), 4: ((1, 1),),
      5: ((0, 0), (0, 1), 1), 6: ((1, 0), (1, 1), 1)}

RC, CW = 8, 256
W0GROUPS = ((0, 1), (1, 2), (2, 4), (4, 8))

def _build():
    w0groups = W0GROUPS
    NW = len(w0groups)
    def kern(x_hbm, wqkv_hbm, wo_hbm, w1_hbm, w3_hbm, w2_hbm, gw_hbm, o_hbm,
             x_v, tk_v, tv_v, wo_v, tq_v, tm_v, t1_v, t3_v, t2_v, xs_v, a_v, g_v, omg_v, macc_v, z_v, kv_v, zacc_v, gw_v, o_v,
             sems, osems):
        sem_next = [0]
        def new_sem():
            sem_next[0] += 1
            return sems.at[sem_next[0] - 1]
        dma = pltpu.make_async_copy
        ds = pl.ds
        x0a = [dma(x_hbm.at[ds(0, 256), :], x_v.at[ds(0, 256), :], new_sem())]
        xcp = [[dma(x_hbm.at[ds(256, 256), :], x_v.at[ds(256, 256), :], new_sem())]]
        xcp += [[dma(x_hbm.at[ds(i * TS1, TS1), :], x_v.at[ds(i * TS1, TS1), :], new_sem())] for i in range(1, N1)]
        ORDER = (0, 4, 1, 5, 2, 6, 3, 7)
        kvcp = []
        for (a0, a1) in w0groups:
            s = new_sem(); cs = []
            for pos in range(a0, a1):
                g = ORDER[pos]; side, p = divmod(g, 4)
                for c0, t_ref in ((D, tk_v), (2 * D, tv_v)):
                    for qr, slot in ((0, (1, 7)[side]), (1, (8, 4)[side])):
                        cs.append(dma(wqkv_hbm.at[ds(qr * D2, D2), ds(c0 + g * 128, 128)], t_ref.at[slot, :, ds(p * 128, 128)], s))
            kvcp.append(cs)
        s_ = new_sem()
        cq = [dma(wqkv_hbm.at[ds(qr * D2, D2), ds(qc * D2, D2)], tq_v.at[slot], s_) for slot, qr, qc in ((1, 0, 0), (2, 0, 1), (3, 1, 0), (4, 1, 1))]
        def blocks(src, dst, kb, nb, part):
            s = new_sem(); hr = kb // 2
            return [dma(src.at[ds(kq * kb + part * hr, hr), ds(nq * nb, nb)], dst.at[slot, ds(part * hr, hr), :], s)
                    for (kq, nq), slot in RAW.items()]
        c1 = [blocks(w1_hbm, t1_v, D4, F4, part) for part in range(2)]
        c3 = [blocks(w3_hbm, t3_v, D4, F4, part) for part in range(2)]
        c2 = [blocks(w2_hbm, t2_v, F4, D4, part) for part in range(2)]
        cwo = [dma(wo_hbm, wo_v, new_sem())]
        cgw = [dma(gw_hbm, gw_v, new_sem())]
        def start(*css):
            for cs in css:
                for c in cs: c.start()
        def wait(*css):
            for cs in css:
                for c in cs: c.wait()
        start(kvcp[0], x0a, xcp[0], *kvcp[1:])
        start(xcp[1], cgw, cq, xcp[2], xcp[3])

        kv_v[...] = jnp.zeros(kv_v.shape, f32)
        zacc_v[...] = jnp.zeros(zacc_v.shape, f32)

        zm = []
        def gate_(v, tk):
            u = pltpu.bitcast(v, u32)
            z = pltpu.bitcast(tk, u32) & zm[0]
            u = u | jnp.tile(z[0:min(8, u.shape[0])], (max(1, u.shape[0] // 8), u.shape[1] // 128))
            return pltpu.bitcast(u, bf16).astype(f32)

        def prep1_task(t_ref, s12, s21, piece):
            r0, nr, c0, nc = piece
            def run(tk):
                ix = lambda slot: (slot, ds(r0, nr), ds(c0, nc))
                tb = b_combos(gate_(t_ref[ix(1)], tk), gate_(t_ref[ix(s12)], tk), gate_(t_ref[ix(s21)], tk), gate_(t_ref[ix(4)], tk))
                for j in (0, 2, 3, 5, 6):
                    t_ref[ix(j)] = tb[j].astype(bf16)
            return run
        def prep2_task(t_ref, r0, c0, i):
            def run(tk):
                ix = lambda slot: (slot, ds(r0, 8), ds(c0, 128))
                q = BQ[i]; l1 = []
                for r in range(2):
                    for c in range(2):
                        a = gate_(t_ref[ix(RAW[2 * q[0][0] + r, 2 * q[0][1] + c])], tk)
                        if len(q) == 3:
                            b = t_ref[ix(RAW[2 * q[1][0] + r, 2 * q[1][1] + c])].astype(f32)
                            a = a + b if q[2] > 0 else a - b
                        l1.append(a)
                for j, v in enumerate(b_combos(*l1)):
                    if i in (1, 4) and j in (1, 4):
                        continue
                    t_ref[ix(7 * i + j)] = v.astype(bf16)
            return run
        def prep2_tasks(t_ref, r0, nrows):
            return [prep2_task(t_ref, r0 + r, c0, i) for r in range(0, nrows, 8) for c0 in range(0, t_ref.shape[-1], 128) for i in range(7)]
        def xs_task(i, r0, c0):
            def run(tk):
                def ld(rr, cc): return gate_(x_v[ds(i * 256 + rr + r0, RC), ds(cc + c0, CW)], tk)
                for j, s_ in enumerate(a_combos(ld(0, 0), ld(0, D2), ld(128, 0), ld(128, D2))):
                    xs_v[i, j, ds(r0, RC), ds(c0, CW)] = s_.astype(bf16)
            return run
        def xs_tasks(t1):
            return [xs_task(2 * t1 + i, r0, c0) for i in range(2) for r0 in range(0, 128, RC) for c0 in range(0, D2, CW)]
        gwl = []
        def gate_task(r0):
            def run(tk):
                rows = ds(r0, 16)
                tot = None
                for g in range(NG):
                    t_ = gate_(x_v[rows, g*128:(g+1)*128], tk) * gwl[0][g:g+1, :]
                    tot = t_ if tot is None else tot + t_
                gt = jnp.broadcast_to(sigmoid(jnp.sum(tot, axis=-1, keepdims=True)), (16, 128))
                g_v[rows, :] = gt
                omg_v[rows, :] = 1.0 - gt
            return run
        def gate_tasks(t1):
            return [gate_task(t1 * TS1 + r) for r in range(0, TS1, 16)]
        TK = [[prep1_task(tk_v, 7, 8, (r, 16, p * 128, 128)) for r in range(0, D2, 16)] for p in range(4)]
        TV = [[prep1_task(tv_v, 7, 8, (r, 16, p * 128, 128)) for r in range(0, D2, 16)] for p in range(4)]
        TQ = [prep1_task(tq_v, 2, 3, (r, RC, c0, CW)) for r in range(0, D2, RC) for c0 in range(0, D2, CW)]
        T1 = [prep2_tasks(t1_v, part * 128, 128) for part in range(2)]
        T3 = [prep2_tasks(t3_v, part * 128, 128) for part in range(2)]
        T2 = [prep2_tasks(t2_v, part * 448, 448) for part in range(2)]

        def spread(tasks, slots):
            out = {g: [] for g in slots}
            for n, t in enumerate(tasks):
                out[slots[n * len(slots) // len(tasks)]].append(t)
            return out
        def mix(*lists):
            tagged = [((n + 0.5) / len(l), k, t) for k, l in enumerate(lists) for n, t in enumerate(l)]
            return [t for _, _, t in sorted(tagged, key=lambda e: e[:2])]
        def run_tasks(tl, results):
            if not tl:
                return
            ticks = [r[a:a + 8, c:c + 128] for r in results for c in range(0, r.shape[1], 128) for a in range(0, r.shape[0], 8)]
            for n_, task in enumerate(tl):
                task(ticks[n_ * len(ticks) // len(tl)])

        def fin(g, k, v):
            pk = phi(k).astype(bf16)
            zacc_v[:, g*128:(g+1)*128] += jnp.sum(pk.astype(f32).reshape(TS1 // 8, 8, 128), axis=0)
            kv_v[g] += jax.lax.dot_general(pk, v.astype(bf16), (((0,), (0,)), ((), ())), preferred_element_type=f32)
        def p1_tile(t, waits, tasks):
            xl = []
            def kvproj(g):
                side, p = divmod(g, 4)
                top, bot = ((1, 8), (7, 4))[side]
                cs = slice(p * 128, (p + 1) * 128)
                wk = cat([tk_v[top, :, cs], tk_v[bot, :, cs]], 0); wv = cat([tv_v[top, :, cs], tv_v[bot, :, cs]], 0)
                if g == ORDER[0]:
                    xa = x_v[0:256, :]
                    ka, va = dot(xa, wk), dot(xa, wv)
                    wait(xcp[0])
                    xb = x_v[256:512, :]
                    xl.append(cat([xa, xb], 0))
                    return cat([ka, dot(xb, wk)], 0), cat([va, dot(xb, wv)], 0)
                return dot(xl[0], wk), dot(xl[0], wv)
            prev = None
            for pos in range(NG):
                if pos in waits:
                    wait(*waits[pos])
                g = ORDER[pos]
                cur = kvproj(g)
                run_tasks(tasks.get(pos, ()), cur)
                if prev is not None:
                    fin(*prev)
                prev = (g,) + cur
            fin(*prev)
        def p1_tile_st(t, tasks):
            xs = [[xs_v[2 * t + i, j] for j in range(7)] for i in range(2)]
            def proj(t_ref, p, tl):
                ms = [[dot(xs[i][j], t_ref[j, :, p*128:(p+1)*128]) for j in range(7)] for i in range(2)]
                run_tasks(tl, ms[0] + ms[1])
                c = [c_combos(m) for m in ms]
                return (cat([c[0][0], c[0][2], c[1][0], c[1][2]], 0), cat([c[0][1], c[0][3], c[1][1], c[1][3]], 0))
            prev = None
            for p in range(4):
                kk = proj(tk_v, p, tasks.get(2 * p, ()))
                if prev is not None:
                    fin(prev[0], prev[1][0], prev[2][0])
                vv = proj(tv_v, p, tasks.get(2 * p + 1, ()))
                if prev is not None:
                    fin(prev[0] + 4, prev[1][1], prev[2][1])
                prev = (p, kk, vv)
            fin(prev[0], prev[1][0], prev[2][0]); fin(prev[0] + 4, prev[1][1], prev[2][1])

        wait(kvcp[0], x0a)
        zm.append((pltpu.bitcast(x_v[0:16, 0:128], u32) >> 31) >> 1)
        W0 = {w0groups[n][0]: [kvcp[n]] for n in range(1, NW)}
        last0 = w0groups[-1][0]
        J8 = list(range(8))
        W0[last0 + 2] = [xcp[1]]
        tk0 = spread(TK[0] + TV[0] + TK[1] + TV[1] + TK[2] + TV[2], list(range(last0, last0 + 2)))
        tk0.update(spread(mix(xs_tasks(1), TK[3] + TV[3]), list(range(last0 + 2, NG))))
        start(c1[0], c1[1])
        p1_tile(0, W0, tk0)
        wait(cgw, cq, xcp[2])
        start(c3[0], c3[1], cwo)
        gwl.append(gw_v[...].astype(f32))
        tk1 = spread(mix(xs_tasks(2), xs_tasks(0), gate_tasks(0) + gate_tasks(1), TQ), J8)
        p1_tile_st(1, tk1)
        wait(xcp[3], c1[0], c1[1])
        start(c2[0], c2[1])
        p1_tile_st(2, spread(mix(xs_tasks(3), gate_tasks(2), T1[0]), J8))
        p1_tile_st(3, spread(mix(gate_tasks(3), T1[1]), J8))

        wait(cwo, c3[0], c3[1])
        r = jax.lax.broadcasted_iota(jnp.int32, (128, 128), 0)
        c = jax.lax.broadcasted_iota(jnp.int32, (128, 128), 1)
        same = (r // DH) == (c // DH)
        def mblk(g):
            kvg = jnp.where(same, kv_v[g], 0.0).astype(bf16)
            return dot(kvg, wo_v[g*128:(g+1)*128, :])
        for g in range(NG):
            zrow = jnp.sum(zacc_v[:, g*128:(g+1)*128], axis=0, keepdims=True)
            zb = jnp.broadcast_to(zrow, (128, 128)).T
            z_v[g] = jnp.where(same, zb, 0.0).astype(bf16)
        for p in range(4):
            mt = mblk(p); mb = mblk(p + 4)
            for j, tb in enumerate(b_combos(mt[:, :D2], mt[:, D2:], mb[:, :D2], mb[:, D2:])):
                tm_v[j, p * 128:(p + 1) * 128, :] = tb.astype(bf16)

        NS = NT * 8
        lt = spread(T3[0] + T3[1], list(range(NS // 2)))
        lt.update(spread(T2[0] + T2[1], list(range(NS // 2, NS))))
        slot_no = [0]
        def tasks_next(ms):
            run_tasks(lt.get(slot_no[0], ()), ms)
            slot_no[0] += 1
            if slot_no[0] == NS // 2:
                wait(c2[0], c2[1])
        def qjob(i, p):
            ms = [dot(xs_v[i, j], tq_v[j, :, p * 128:(p + 1) * 128]) for j in range(7)]
            tasks_next(ms)
            return c_combos(ms)
        def denjob(p, q4):
            out = []
            for k, q in enumerate(q4):
                pq = phi(q)
                out.append((pq, dot(pq.astype(bf16), z_v[p + 4 * (k % 2)]) + 1e-6))
            return out
        def norm(i, pd):
            gts = (g_v[i * 256:i * 256 + 128, :], g_v[i * 256 + 128:(i + 1) * 256, :])
            return [s.astype(bf16) for s in a_combos(*[pq * (gts[k // 2] * rcp(den)) for k, (pq, den) in enumerate(pd)])]
        def ajob(i, ss):
            lhs = [cat([ss[p][j] for p in range(4)]) for j in range(7)]
            for n in range(4):
                cs = slice(n * 128, (n + 1) * 128)
                ms = [dot(lhs[j], tm_v[j, :, cs]) for j in range(7)]
                tasks_next(ms)
                c11, c12, c21, c22 = c_combos(ms)
                r0 = i * 256
                a_v[r0:r0 + 128, n*128:(n+1)*128] = c11.astype(bf16)
                a_v[r0:r0 + 128, D2 + n*128:D2 + (n+1)*128] = c12.astype(bf16)
                a_v[r0 + 128:r0 + 256, n*128:(n+1)*128] = c21.astype(bf16)
                a_v[r0 + 128:r0 + 256, D2 + n*128:D2 + (n+1)*128] = c22.astype(bf16)
        prev_q = None; prev_ss = None
        for i in range(NT):
            q = [None] * 4; ss = [None] * 4
            q[0] = qjob(i, 0)
            if i > 0:
                prev_ss[3] = norm(i - 1, denjob(3, prev_q))
            q[1] = qjob(i, 1); pd0 = denjob(0, q[0])
            if i > 0:
                ajob(i - 1, prev_ss)
            ss[0] = norm(i, pd0)
            q[2] = qjob(i, 2); ss[1] = norm(i, denjob(1, q[1]))
            q[3] = qjob(i, 3); ss[2] = norm(i, denjob(2, q[2]))
            prev_q, prev_ss = q[3], ss
        prev_ss[3] = norm(NT - 1, denjob(3, prev_q))
        ajob(NT - 1, prev_ss)

        def ocp(slot, i):
            return dma(o_v.at[slot], o_hbm.at[ds(pl.multiple_of(i * 256, 256), 256), :], osems.at[slot])

        def p2(i, _):
            slot = i % 2
            @pl.when(i >= 2)
            def _():
                ocp(slot, i - 2).wait()
            r0 = pl.multiple_of(i * 256, 256)
            oms = [omg_v[ds(r0 + rb * 64, 64), :] for rb in range(4)]
            xb = {(rb, kq): x_v[ds(r0 + rb * 64, 64), kq * D4:(kq + 1) * D4].astype(f32) for rb in range(4) for kq in range(4)}
            x2 = [v.astype(bf16) for v in combos2(a_combos, xb)]
            def f2(t_ref, p):
                return c_combos2([dot(x2[s], t_ref[s, :, p*128:(p+1)*128]) for s in range(49)])
            def gujob(p):
                return f2(t1_v, p), f2(t3_v, p)
            def gufin(gu):
                g, u = gu
                h = {k: (g[k] * sigmoid(g[k])) * (u[k] * oms[k[0]]) for k in g}
                return [s.astype(bf16) for s in combos2(a_combos, h)]
            gu = {}; sh = {}
            def l2(ps, first):
                for s in range(49):
                    d = dot(cat([sh[p][s] for p in ps]), t2_v[s, ps[0] * 128:(ps[-1] + 1) * 128, :])
                    macc_v[s] = d if first else macc_v[s] + d
            gu[0] = gujob(0)
            for p in (1, 2, 3, 4):
                gu[p] = gujob(p); sh[p - 1] = gufin(gu[p - 1])
            l2((0, 1, 2), True)
            for p in (5, 6):
                gu[p] = gujob(p); sh[p - 1] = gufin(gu[p - 1])
            l2((3, 4, 5), False)
            sh[6] = gufin(gu[6])
            for n in range(2):
                cs = slice(n * 128, (n + 1) * 128)
                ms = [macc_v[s, :, cs] + dot(sh[6][s], t2_v[s, 768:896, cs]) for s in range(49)]
                for (rb, nq), cblk in c_combos2(ms).items():
                    cols = slice(nq * D4 + n * 128, nq * D4 + (n + 1) * 128)
                    o_v[slot, rb * 64:(rb + 1) * 64, cols] = (cblk + a_v[ds(r0 + rb * 64, 64), cols].astype(f32)).astype(bf16)
            ocp(slot, i).start()
            return 0
        jax.lax.fori_loop(0, NT, p2, 0)
        ocp((NT - 2) % 2, NT - 2).wait()
        ocp((NT - 1) % 2, NT - 1).wait()

    def fn(A_x, A_wqkv, A_wo, B_x, B_w1, B_w3, B_w2, gate_w):
        x2 = A_x.reshape(S, D)
        gw = gate_w.reshape(NG, 128)
        any_ = pl.BlockSpec(memory_space=pl.ANY)
        V = pltpu.VMEM
        out = pl.pallas_call(
            kern,
            in_specs=[any_] * 7,
            out_specs=any_,
            out_shape=jax.ShapeDtypeStruct((S, D), bf16),
            scratch_shapes=[
                V((S, D), bf16), V((9, D2, D2), bf16), V((9, D2, D2), bf16), V((D, D), bf16),
                V((7, D2, D2), bf16), V((7, D2, D2), bf16),
                V((49, D4, F4), bf16), V((49, D4, F4), bf16), V((49, F4, D4), bf16),
                V((NT, 7, 128, D2), bf16), V((S, D), bf16), V((S, 128), f32), V((S, 128), f32),
                V((49, 64, D4), f32), V((NG, 128, 128), bf16), V((NG, 128, 128), f32),
                V((8, D), f32), V((NG, 128), bf16), V((2, 256, D), bf16),
                pltpu.SemaphoreType.DMA((N1 + NW + 10,)), pltpu.SemaphoreType.DMA((2,)),
            ],
            compiler_params=pltpu.CompilerParams(vmem_limit_bytes=126 * 1024 * 1024),
        )(x2, A_wqkv, A_wo, B_w1, B_w3, B_w2, gw)
        return out.reshape(1, S, D)
    return fn


_impl = _build()


@jax.jit
def pallas_gated_mix__linear_attn_block__glu_gated_swiglu__prompt_kernel(A_x, A_wqkv, A_wo, B_x, B_w1, B_w3, B_w2, gate_w):
    return _impl(A_x, A_wqkv, A_wo, B_x, B_w1, B_w3, B_w2, gate_w)
```
